```python
import os as _os
_os.environ.setdefault("JAX_PLATFORMS", "cpu")
import jax
import jax.numpy as jnp

def _softmax(x, axis=-1):
    return jax.nn.softmax(x, axis=axis)
def _gelu(x):
    return jax.nn.gelu(x, approximate=True)
def _silu(x):
    return jax.nn.silu(x)
def _sigmoid(x):
    return jax.nn.sigmoid(x)
def _layernorm(x, axis=-1, eps=1e-5):
    m = jnp.mean(x, axis=axis, keepdims=True)
    v = jnp.var(x, axis=axis, keepdims=True)
    return (x - m) / jnp.sqrt(v + eps)
def _scatter_add(tgt, idx, src, axis=0):
    return tgt.at[idx].add(src)
def _segment_sum(src, seg, n):
    return jax.ops.segment_sum(src, seg, n)
class _Rng:
    def __init__(self, key):
        self._k = key
    def _next(self):
        self._k, sub = jax.random.split(self._k)
        return sub
    def normal(self, shape):
        return jax.random.normal(self._next(), shape, dtype=jnp.bfloat16)
    def randint(self, lo, hi, shape):
        return jax.random.randint(self._next(), shape, lo, hi, dtype=jnp.int32)
    def uniform(self, shape, lo=0.0, hi=1.0):
        return jax.random.uniform(self._next(), shape, jnp.bfloat16, lo, hi)
    def permutation(self, n):
        return jax.random.permutation(self._next(), n)


kernel_name = 'gated_mix__ssm_conv_h3__linear_kernel_hedgehog__prompt'

def setup_inputs():
    _rng = _Rng(jax.random.key(int.from_bytes(__import__("os").urandom(4), "little")))
    _w = (lambda a: (lambda t: t.astype(jnp.bfloat16) if jnp.issubdtype(t.dtype, jnp.floating) else t)(jnp.asarray(a)))
    def _A_setup():
        B, S, D = 1, 2048, 576
        ks = 4
        return {
            "q": _w((lambda *s: _rng.normal(s) * 0.05)(B, S, D)),
            "k": _w((lambda *s: _rng.normal(s) * 0.4)(B, S, D)),
            "v": _w((lambda *s: _rng.normal(s) * 0.4)(B, S, D)),
            "shift_k": _w((lambda *s: _rng.normal(s) * 0.4)(D, ks) * 0.5),
            "ssm_k": _w((lambda *s: _rng.normal(s) * 0.4)(D, S) * (1.0 / S ** 0.5)),
            "ssm_D": _w((lambda *s: _rng.normal(s) * 0.4)(D)),
        }
    _A_in = _A_setup()

    def _B_setup():
        B, S, D, H = 1, 2048, 576, 32
        Dh = D // H
        return {
            "x": _w((lambda *s: _rng.normal(s) * 0.05)(B, S, D)),
            "wqkv": _w((lambda *s: _rng.normal(s) * 0.8)(D, 3 * D)),
            "w_phi": _w((lambda *s: _rng.normal(s) * 0.8)(H, Dh, Dh) * (Dh ** -0.5)),
            "wo": _w((lambda *s: _rng.normal(s) * 0.05)(D, D)),
        }
    _B_in = _B_setup()

    return {
        "A_q": _A_in["q"],
        "A_k": _A_in["k"],
        "A_v": _A_in["v"],
        "A_shift_k": _A_in["shift_k"],
        "A_ssm_k": _A_in["ssm_k"],
        "A_ssm_D": _A_in["ssm_D"],
        "B_x": _B_in["x"],
        "B_wqkv": _B_in["wqkv"],
        "B_w_phi": _B_in["w_phi"],
        "B_wo": _B_in["wo"],
        "gate_w": _w((lambda *s: _rng.normal(s) * 0.05)(576) * 16.0),
    }

def reference(A_q, A_k, A_v, A_shift_k, A_ssm_k, A_ssm_D, B_x, B_wqkv, B_w_phi, B_wo, gate_w):
    def _A_ref(q, k, v, shift_k, ssm_k, ssm_D):
        B, S, D = q.shape
        ks = shift_k.shape[-1]
        k_pad = jnp.pad(k, ((0, 0), (ks - 1, 0), (0, 0)))
        k_shift = jnp.zeros_like(k)
        for t in range(ks):
            k_shift = k_shift + k_pad[:, t:t + S, :] * shift_k[:, ks - 1 - t][None, None, :]
        kv = k_shift * v
        L = 2 * S
        kv_pad = jnp.pad(kv, ((0, 0), (0, S), (0, 0)))
        kf_pad = jnp.pad(ssm_k, ((0, 0), (0, S)))
        kv_f = (lambda x, axes=(-2,-1): jnp.fft.rfft2(x.astype(jnp.float32), axes=axes))(kv_pad[:, None, :, :], axes=(1, 2))
        kf_f = (lambda x, axes=(-2,-1): jnp.fft.rfft2(x.astype(jnp.float32), axes=axes))(kf_pad[:, None, :], axes=(1, 2))
        kf_f = (lambda x, *d: x.transpose(*d))(kf_f, 1, 2, 0)
        y_f = kv_f * kf_f[None, :, :, :]
        y = (lambda x, s, axes=(-2,-1): jnp.fft.irfft2(x, s=s, axes=axes).astype(jnp.bfloat16))(y_f, (1, L), axes=(1, 2))[:, 0, :S, :]
        y = y + kv * ssm_D[None, None, :]
        return q * y

    def _B_ref(x, wqkv, w_phi, wo):
        B, S, D = x.shape
        H = 32; Dh = D // H
        qkv = (lambda x, *d: x.transpose(*d))((x @ wqkv).reshape(B, S, 3, H, Dh), 2, 0, 3, 1, 4)
        q, k, v = qkv[0], qkv[1], qkv[2]
        pq = jnp.einsum("bhsd,hdf->bhsf", q, w_phi)
        pk = jnp.einsum("bhsd,hdf->bhsf", k, w_phi)
        phi_q = jnp.concatenate([_softmax(pq, axis=-1), _softmax(-pq, axis=-1)], axis=-1)
        phi_k = jnp.concatenate([_softmax(pk, axis=-1), _softmax(-pk, axis=-1)], axis=-1)
        kv = jnp.einsum("bhsf,bhsd->bhfd", phi_k, v)
        z  = jnp.einsum("bhsf->bhf", phi_k)
        num = jnp.einsum("bhqf,bhfd->bhqd", phi_q, kv)
        den = jnp.einsum("bhqf,bhf->bhq", phi_q, z)[..., None] + 1e-6
        o = num / den
        return (lambda x, *d: x.transpose(*d))(o, 0, 2, 1, 3).reshape(B, S, D) @ wo

    x = A_q
    g = _sigmoid((x * gate_w).sum(-1, keepdims=True))
    a = _A_ref(x, A_k, A_v, A_shift_k, A_ssm_k, A_ssm_D)
    b = _B_ref(x, B_wqkv, B_w_phi, B_wo)
    return g * a + (1 - g) * b
```

```python
import math

import jax
import jax.numpy as jnp
import numpy as np
import jax.experimental.pallas as pl
import jax.experimental.pallas.tpu as pltpu

S = 2048
D = 576
NH = 32
DH = 18
NG = 8
GR = 72
NC = 16
NIT = 4
CH = S // NIT
CB = 8
RO = 32
A_ROWS = (0, 160, 368, 576)
C_ROWS = (0, 32, 64, 512, 576)
RB = (C_ROWS[3] - C_ROWS[2]) // NIT
PW_QT, PW_Q, PW_N, PW_W, PW_WT = 1.1, (0, 0, 0, 0), (0, 0, 0.5, 0.5), (0.9, 0.9, 1.0, 1.0), 1.1
PB_VT, PB_V, PB_X, PB_KT, PB_K, PB_H = 1.5, (1.0,) * 4, 0, 1.2, (0,) * 4, 0

F32 = jnp.float32
BF16 = jnp.bfloat16
_NN = (((1,), (0,)), ((), ()))
_NT = (((1,), (1,)), ((), ()))
LOG2E = math.log2(math.e)


def _dot(a, b, dn=_NN):
    return jax.lax.dot_general(a, b, dn, preferred_element_type=F32)


def _eps(c):
    return 1 if (c // 2) % 2 == 0 else -1


def _iota(shape, dim):
    return jax.lax.broadcasted_iota(jnp.int32, shape, dim)


def _cat(xs, axis=0):
    return jnp.concatenate(xs, axis=axis)


def _pk(x):
    return pltpu.bitcast(x, jnp.uint32)


def _upk(x):
    return pltpu.bitcast(x, BF16)


def _rcp(x):
    return pl.reciprocal(x, approx=True)


def _dft_table():
    om = np.pi * (2 * np.arange(128) + 1) / 256.0
    tau = np.arange(256)
    ang = np.outer(tau, om)
    return np.concatenate([np.cos(ang), -np.sin(ang)], axis=1).astype(np.float32)


class _Pacer:
    def __init__(self, mask):
        self.mask = mask
        self.runs = [[]]
        self.len = [0.0]

    def add(self, arr, cycles, w=1.0):
        if w == 0:
            if self.runs[-1]:
                self.runs.append([])
                self.len.append(0.0)
            return
        cycles = cycles * w
        n = arr.shape[0] // 8
        for r in range(n):
            self.runs[-1].append((self.len[-1] + cycles * r / n, arr[8 * r:8 * r + 8, 0:128]))
        self.len[-1] += cycles

    def plan(self, sizes):
        tot, cap = float(sum(sizes)), sum(self.len)
        edges, acc = [], 0.0
        for ln in self.len:
            acc += ln
            edges.append(acc / cap * tot)
        self.unit_run, done = [], 0.0
        self.load = [0.0] * len(self.runs)
        for sz in sizes:
            r = min(i for i, e in enumerate(edges) if done + sz / 2 <= e + 1e-6)
            self.unit_run.append(r)
            self.load[r] += sz
            done += sz
        self.used = [0.0] * len(self.runs)
        self.unit = -1

    def next_unit(self):
        self.unit += 1

    def gate(self, x, nops):
        r = self.unit_run[self.unit]
        t = self.len[r] * self.used[r] / self.load[r]
        self.used[r] += nops
        tok = [v for tt, v in self.runs[r] if tt <= t][-1]
        return jnp.where(self.mask, x, tok)


class _NoPacer:
    def add(self, arr, cycles, w=1.0):
        pass


def _red(op, vs, lo2):
    rab = op(op(vs[0], vs[1]), op(vs[2], vs[3]))
    rcd = op(op(vs[4], vs[5]), op(vs[6], vs[7]))
    a = jnp.where(lo2, rab, rcd)
    b = jnp.where(lo2, rcd, rab)
    m = op(op(a, pltpu.roll(b, 2, 0)), vs[8])
    return op(m, pltpu.roll(m, 4, 0))


def _expand(m, lo2):
    r = pltpu.roll(m, 2, 0)
    ab = jnp.where(lo2, m, r)
    cd = jnp.where(lo2, r, m)
    return [ab] * 4 + [cd] * 4 + [m]


def _feature_map(p, lo2, normalize):
    vs = [p[8 * j:8 * j + 8] for j in range(9)]
    mx = _expand(_red(jnp.maximum, vs, lo2), lo2)
    mn = _expand(_red(jnp.minimum, vs, lo2), lo2)
    ep = [jnp.exp2(v - m) for v, m in zip(vs, mx)]
    em = [jnp.exp2(m - v) for v, m in zip(vs, mn)]
    sp = _red(jnp.add, ep, lo2)
    sm = _red(jnp.add, em, lo2)
    if normalize:
        ep = [e * r for e, r in zip(ep, _expand(_rcp(sp), lo2))]
        em = [e * r for e, r in zip(em, _expand(_rcp(sm), lo2))]
    else:
        em = [e * r for e, r in zip(em, _expand(sp * _rcp(sm), lo2))]
    shared = _cat([ep[8], em[8]]).astype(BF16)
    return (_cat([_cat(ep[0:4] + em[0:4]).astype(BF16), shared]),
            _cat([_cat(ep[4:8] + em[4:8]).astype(BF16), shared]))


def _kernel(q_hbm, k_hbm, v_hbm, h_hbm, w_hbm, wo_hbm,
            sk_hbm, dd_hbm, gw_hbm, wp_hbm, ft_hbm, zero_hbm,
            out_hbm,
            q_v, k_v, v_v, h_v, w_v, wo_v, sk_ref, dd_ref, gw_ref, wp_ref, ft_ref, zero_s,
            wkv_t, wq_t, wo_t,
            x3a, x3b, x3c, x3d, h3a, h3b, h3c, h3d, y2, y2d, kvacc, kvt, b_t, g8, o_v, cb,
            sems):
    x3s = (x3a, x3b, x3c, x3d)
    h3s = (h3a, h3b, h3c, h3d)

    def cp(src, dst, i):
        return pltpu.make_async_copy(src, dst, sems.at[i])

    def cq(i, s):
        return cp(q_hbm.at[:, CH * i:CH * (i + 1)], q_v.at[:, CH * i:CH * (i + 1)], s)

    def ca(i, s):
        rows = slice(A_ROWS[i], A_ROWS[i + 1])
        return [cp(h_hbm.at[rows, :], h_v.at[rows, :], s),
                cp(k_hbm.at[rows, :], k_v.at[rows, :], s),
                cp(v_hbm.at[rows, :], v_v.at[rows, :], s)]

    sets = [
        [cp(wp_hbm, wp_ref, 0)],
        [cp(w_hbm.at[:, 512:1152], w_v.at[:, 512:1152], 1)],
        [cq(0, 2), cp(sk_hbm, sk_ref, 2), cp(dd_hbm, dd_ref, 2), cp(gw_hbm, gw_ref, 2),
         cp(zero_hbm, zero_s, 2)],
        [cp(w_hbm.at[:, 1152:1728], w_v.at[:, 1152:1728], 3),
         cp(w_hbm.at[:, 0:512], w_v.at[:, 0:512], 3)],
        [cq(1, 4), cp(ft_hbm, ft_ref, 4)] + ca(0, 4),
        [cq(2, 5), cp(wo_hbm, wo_v, 5)] + ca(1, 5),
        [cq(3, 6)] + ca(2, 6),
    ]

    def c_out(i):
        return cp(o_v.at[RO * i:RO * (i + 1), :], out_hbm.at[RO * i:RO * (i + 1), :], 0)

    def wait(i):
        for c in sets[i]:
            c.wait()

    for i, cs in enumerate(sets):
        for c in cs:
            c.start(priority=0 if i < 2 else 1)
    wait(0)

    def row_maps(shape):
        r = _iota(shape, 0)
        j, s = r // 8, r % 8
        feat = jnp.where(j < 8, 4 * (j % 4) + s // 2, 16 + s // 4)
        head = jnp.where(j < 8, 2 * (j // 4) + s % 2, s % 4)
        return feat, head

    col = _iota((NH, 640), 1)
    hrow = _iota((NH, 640), 0) * DH
    wt = jnp.zeros((DH, 640), F32)
    for d in range(DH):
        sel = jnp.where(col == hrow + d, 1.0, 0.0).astype(BF16)
        wt = wt + _dot(wp_ref[d], sel)
    rsel = jnp.where(row_maps((GR, DH))[0] == _iota((GR, DH), 1), 1.0, 0.0).astype(BF16)
    z0 = _dot(rsel, wt.astype(BF16))
    z64 = pltpu.roll(z0, 64, 1)

    zrel = _iota((GR, 128), 1) - DH * row_maps((GR, 128))[1]

    def fold(z, off, base, g):
        lo = off + GR * g
        t0, t1 = lo // 128, (lo + GR - 1) // 128 + 1
        es = []
        for t in range(t0, t1):
            rel = zrel + (128 * t - lo)
            m = jnp.logical_and(rel >= 0, rel < DH)
            es.append(jnp.where(m, z[:, 128 * t:128 * t + 128], 0.0))
        e = _cat(es, 1).astype(BF16)
        return _dot(e, w_v[:, base + 128 * t0: base + 128 * t1], _NT) * LOG2E

    wait(1)
    for p in range(NG // 2):
        r = _cat([fold(z64, 64, 512, 2 * p), fold(z64, 64, 512, 2 * p + 1)])
        wkv_t[GR * p: GR * (p + 1), :] = _pk(r.astype(BF16))

    lane = _iota((16, 128), 1)
    sub8 = _iota((8, 128), 0)
    lo2 = sub8 % 4 < 2
    top = sub8 < 4

    def proj_steps(w_t, r0, r1, c0, pacer, wt_=1.0, wm=(1.0,) * 4):
        m = 2 * (r1 - r0)
        tail = _dot(_upk(w_t[r0:r1, 512:D]), q_v[512:D, pl.ds(c0, CH)])
        pacer.add(tail, m, wt_)
        yield None
        for n in range(CH // 128):
            cn = c0 + 128 * n
            if not isinstance(cn, int):
                cn = pl.multiple_of(cn, 128)
            pm_ = _dot(_upk(w_t[r0:r1, 0:512]), q_v[0:512, pl.ds(cn, 128)])
            pacer.add(pm_, m, wm[n])
            yield pm_ + tail[:, 128 * n:128 * n + 128]

    def k_feat(pk):
        out = []
        for g in range(NG):
            out += list(_feature_map(pk[GR * g: GR * (g + 1)], lo2, True))
        return out

    ones8 = jnp.ones((8, 128), F32)

    def v_ext(pv):
        out = []
        for g in range(NG):
            out.append(_cat([pv[GR * g: GR * g + 40], ones8]).astype(BF16))
            out.append(_cat([pv[GR * g + 32: GR * g + 72], ones8]).astype(BF16))
        return out

    def kv_step(acc, phi, vx):
        r = [_dot(vx[p], phi[p], _NT) for p in range(2 * NG)]
        return r if acc is None else [a + b for a, b in zip(acc, r)]

    def spec_ref(refs, row):
        for i in range(4):
            if row < C_ROWS[i + 1]:
                if i < 2:
                    return refs[i], pl.ds(pl.multiple_of(zero_s[0] + (row - C_ROWS[i]), 16), 16)
                return refs[i], pl.ds(row - C_ROWS[i], 16)

    def h_spec(rows16, pacer):
        le, lo_ = [], []
        for r in rows16:
            for c in range(NC):
                (le if c % 2 == 0 else lo_).append(h_v[r:r + 16, 128 * c:128 * c + 128])
        he = _dot(_cat(le), ft_ref[0:128, :])
        ho = _dot(_cat(lo_), ft_ref[128:256, :])
        pacer.add(he, 64 * len(rows16), PB_H)
        pacer.add(ho, 64 * len(rows16), PB_H)
        for sb, r in enumerate(rows16):
            ref, rr = spec_ref(h3s, r)
            prev = None
            for c in range(NC):
                o = (sb * (NC // 2) + c // 2) * 16
                hh = (he if c % 2 == 0 else ho)[o:o + 16]
                if prev is None:
                    cc = hh[:, 0:128] + cb[4, r:r + 16, :]
                    dd_ = hh[:, 128:256]
                else:
                    hp = hh + prev if _eps(c) * _eps(c - 1) > 0 else hh - prev
                    cc = hp[:, 0:128]
                    dd_ = hp[:, 128:256]
                prev = hh
                ref[rr, 384 * c: 384 * c + 128] = cc
                ref[rr, 384 * c + 128: 384 * c + 256] = cc + dd_
                ref[rr, 384 * c + 256: 384 * c + 384] = dd_ - cc

    def x_spec(rows16, pacer):
        le, lo_ = [], []
        for r in rows16:
            s0, s1, s2, s3 = (cb[j, r:r + 16, :] for j in range(4))
            pr1 = None
            pr2 = None
            for c in range(NC):
                cs = slice(128 * c, 128 * c + 128)
                kf = k_v[r:r + 16, cs].astype(F32)
                r1 = pltpu.roll(kf, 1, 1)
                k1 = jnp.where(lane >= 1, r1, 0.0 if pr1 is None else pr1)
                pr1 = r1
                w1 = s0 * kf + s1 * k1
                w2 = s2 * kf + s3 * k1
                r2 = pltpu.roll(w2, 2, 1)
                k2 = jnp.where(lane >= 2, r2, 0.0 if pr2 is None else pr2)
                pr2 = r2
                kv = ((w1 + k2) * v_v[r:r + 16, cs].astype(F32)).astype(BF16)
                (le if c % 2 == 0 else lo_).append(kv)
        xe = _dot(_cat(le), ft_ref[0:128, :])
        xo = _dot(_cat(lo_), ft_ref[128:256, :])
        pacer.add(xe, 64 * len(rows16), PB_X)
        pacer.add(xo, 64 * len(rows16), PB_X)
        for sb, r in enumerate(rows16):
            ref, rr = spec_ref(x3s, r)
            for c in range(NC):
                o = (sb * (NC // 2) + c // 2) * 16
                xx = (xe if c % 2 == 0 else xo)[o:o + 16]
                xa = xx[:, 0:128]
                xb = xx[:, 128:256]
                ref[rr, 384 * c: 384 * c + 128] = xa + xb
                ref[rr, 384 * c + 128: 384 * c + 256] = xb
                ref[rr, 384 * c + 256: 384 * c + 384] = xa

    def conv(x3, h3, r_in, r_out, ntask, pacer, y2=y2):
        pacer.plan([3 * CB * (2 * t0 + CB + 1) for t0 in range(0, NC, CB)] * ntask)
        for tk in range(ntask):
            rows = pl.ds(r_in + 8 * tk if isinstance(r_in, int) else pl.multiple_of(r_in + 8 * tk, 8), 8)
            orow = pl.ds(pl.multiple_of(r_out + 8 * tk, 8), 8)
            for t0 in range(0, NC, CB):
                pacer.next_unit()
                k1 = None
                for comp in range(3):
                    def ld(ref, j):
                        return ref[rows, 384 * j + 128 * comp: 384 * j + 128 * comp + 128]
                    hh = {}
                    acc = {} if comp == 0 else dict(k1)
                    for s in range(t0 + CB):
                        ts = [t for t in range(t0, t0 + CB) if t >= s]
                        x = pacer.gate(ld(x3, s), 2 * len(ts))
                        for t in ts:
                            j = t - s
                            if j not in hh:
                                hh[j] = ld(h3, j)
                            sg = _eps(s) * _eps(j) * _eps(t) * (-1 if comp == 1 else 1)
                            prod = x * hh[j]
                            if t not in acc:
                                acc[t] = prod
                            elif sg > 0:
                                acc[t] = acc[t] + prod
                            else:
                                acc[t] = acc[t] - prod
                        if comp > 0 and s >= t0:
                            y2[orow, 256 * s + 128 * (comp - 1): 256 * s + 128 * comp] = acc[s]
                    if comp == 0:
                        k1 = acc

    def true_mask():
        return jnp.abs(ft_ref[0:16, 0:128].astype(F32)[0:8]) < 2.0

    nop = _NoPacer()

    wait(2)
    phis = [k_feat(pk) for pk in list(proj_steps(wkv_t, 0, D // 2, 0, nop))[1:]]
    sk = sk_ref[...].astype(F32)
    for j in range(4):
        cb[j] = jnp.broadcast_to(sk[j:j + 1, :], (128, D)).T
    dd = dd_ref[...].astype(F32).reshape(1, D)
    cb[4] = jnp.broadcast_to(dd, (128, D)).T

    wait(3)
    wkv_t[D // 2:D, :] = _pk(w_v[:, 2 * D:3 * D].T)
    for p in range(NG // 2):
        r = _cat([fold(z0, 0, 0, 2 * p), fold(z0, 0, 0, 2 * p + 1)])
        wq_t[GR * p: GR * (p + 1), :] = _pk(r.astype(BF16))
    wq_t[D // 2:D // 2 + 8, :] = _pk(jnp.broadcast_to(gw_ref[...].reshape(1, D), (16, D)))
    vxs = [v_ext(pv) for pv in list(proj_steps(wkv_t, D // 2, D, 0, nop))[1:]]
    for p in range(2 * NG):
        kvacc[p] = _dot(_cat([v[p] for v in vxs], 1), _cat([f[p] for f in phis], 1), _NT)

    for b in range(3):
        wait(4 + b)
        ntask = (C_ROWS[b] - C_ROWS[b - 1]) // 8 if b > 0 else 0
        pacer = _Pacer(true_mask()) if ntask else nop
        r16 = list(range(A_ROWS[b], A_ROWS[b + 1], 16))
        parts = [r16[(len(r16) * n) // 4: (len(r16) * (n + 1)) // 4] for n in range(4)]
        vs = proj_steps(wkv_t, D // 2, D, CH * (b + 1), pacer, PB_VT, PB_V)
        ks = proj_steps(wkv_t, 0, D // 2, CH * (b + 1), pacer, PB_KT, PB_K)
        next(vs)
        vxs = [v_ext(next(vs))]
        for n in range(3):
            vxs.append(v_ext(next(vs)))
            x_spec(parts[n], pacer)
        next(ks)
        x_spec(parts[3], pacer)
        acc = None
        phi = None
        for n in range(4):
            nxt = k_feat(next(ks))
            if n > 0:
                acc = kv_step(acc, phi, vxs[n - 1])
            phi = nxt
            h_spec(parts[n], pacer)
        acc = kv_step(acc, phi, vxs[3])
        for p in range(2 * NG):
            kvacc[p] += acc[p]
        if b == 1:
            wo_t[...] = _pk(wo_v[...].T)
        if ntask:
            conv(x3s[b - 1], h3s[b - 1], 0, zero_s[0] + C_ROWS[b - 1], ntask, pacer)

    kr = _iota((48, 80), 0)
    kc = _iota((48, 80), 1)
    plus = jnp.logical_or(kc < 32, jnp.logical_and(kc >= 64, kc < 72))
    epsm = jnp.where(jnp.logical_and(kr >= 40, plus), 1e-6, 0.0)
    for pp in range(2):
        rv = kr - 4 * pp
        rhead = jnp.where(kr >= 40, (kr - 40) // 4, jnp.where(rv >= DH, 1, 0))
        rok = jnp.logical_or(kr >= 40, jnp.logical_and(rv >= 0, rv < 2 * DH))
        cok = jnp.logical_or(kc < 64, (kc % 4) // 2 == pp)
        keep = jnp.logical_and(jnp.logical_and(rok, cok), rhead == kc % 2)
        for g in range(NG):
            p = 2 * g + pp
            kvt[p] = _pk(jnp.where(keep, kvacc[p] + epsm, 0.0).astype(BF16))

    def loop2(i, carry):
        c0 = pl.multiple_of(i * CH, CH)
        pacer = _Pacer(true_mask())

        def sub(n):
            return pl.ds(pl.multiple_of(c0 + 128 * n, 128), 128)

        def numden(n, pq):
            g = 1.0 / (1.0 + jnp.exp(-pq[D:D + 8]))
            g8[:, sub(n)] = g * (1.0 / 128.0)
            omg = 1.0 - g
            os = []
            for gi in range(NG):
                tiles = _feature_map(pq[GR * gi: GR * (gi + 1)], lo2, False)
                res = []
                for pp in range(2):
                    a = _dot(_upk(kvt[2 * gi + pp]), tiles[pp])
                    if pp == 1 and gi % 2 == 1:
                        pacer.add(a, 48, PW_N[n])
                    r = omg * _rcp(a[40:48])
                    r4 = pltpu.roll(r, 4, 0)
                    ra = jnp.where(top, r, r4)
                    rb = jnp.where(top, r4, r)
                    mix = jnp.where(sub8 < 2 + 4 * pp, ra, rb)
                    res.append([a[8 * j:8 * j + 8] * s for j, s in enumerate((ra, ra, mix, rb, rb))])
                os += res[0][0:4] + [res[0][4] + res[1][0]] + res[1][1:5]
            return _cat(os[0:64]).astype(BF16), _cat(os[64:72]).astype(BF16)

        def womain(n, o):
            bb = _dot(_upk(wo_t[:, 0:512]), o[0])
            pacer.add(bb, 576, PW_W[n])
            return bb

        qs = proj_steps(wq_t, 0, D // 2 + 8, c0, pacer, PW_QT, PW_Q)
        next(qs)
        pq0 = next(qs)
        pq1 = next(qs)
        o0 = numden(0, pq0)
        pq2 = next(qs)
        o1 = numden(1, pq1)
        b0 = womain(0, o0)
        pq3 = next(qs)
        o2 = numden(2, pq2)
        b1 = womain(1, o1)
        o3 = numden(3, pq3)
        b2 = womain(2, o2)
        btail = _dot(_upk(wo_t[:, 512:D]), _cat([o[1] for o in (o0, o1, o2, o3)], 1))
        pacer.add(btail, 576, PW_WT)
        b3 = womain(3, o3)
        for n, bb in enumerate((b0, b1, b2, b3)):
            b_t[:, sub(n)] = bb + btail[:, 128 * n:128 * n + 128]

        conv(x3c, h3c, i * RB, i * RB + C_ROWS[2], RB // 8, pacer)
        return carry

    jax.lax.fori_loop(0, NIT, loop2, 0)

    pacer = _Pacer(true_mask())
    for i in range(D // RO):
        rows = slice(RO * i, RO * (i + 1))
        if RO * i == C_ROWS[3]:
            z = zero_s[0]
            conv(x3d, h3d, 0, z, (C_ROWS[4] - C_ROWS[3]) // 8, pacer, y2d)
        ysrc, yr = (y2, rows) if RO * i < C_ROWS[3] else (y2d, slice(RO * i - C_ROWS[3], RO * (i + 1) - C_ROWS[3]))
        ye = _cat([ysrc[yr, 512 * c: 512 * c + 256] for c in range(NC // 2)])
        yo = _cat([ysrc[yr, 512 * c + 256: 512 * c + 512] for c in range(NC // 2)])
        te = _dot(ye.astype(BF16), ft_ref[0:128, :], _NT)
        to = _dot(yo.astype(BF16), ft_ref[128:256, :], _NT)
        if RO * (i + 2) <= C_ROWS[3]:
            pacer.add(to, 8 * RO)
        for c in range(NC):
            cs = slice(128 * c, 128 * c + 128)
            y = (te if c % 2 == 0 else to)[(c // 2) * RO: (c // 2 + 1) * RO]
            gq = q_v[rows, cs].astype(F32) * _cat([g8[:, cs]] * (RO // 8))
            o_v[rows, cs] = (gq * y + b_t[rows, cs]).astype(BF16)
        c_out(i).start()
    for i in range(D // RO):
        c_out(i).wait()


@jax.jit
def pallas_gated_mix__ssm_conv_h3__linear_kernel_hedgehog__prompt_kernel(
    A_q: jax.Array,
    A_k: jax.Array,
    A_v: jax.Array,
    A_shift_k: jax.Array,
    A_ssm_k: jax.Array,
    A_ssm_D: jax.Array,
    B_x: jax.Array,
    B_wqkv: jax.Array,
    B_w_phi: jax.Array,
    B_wo: jax.Array,
    gate_w: jax.Array,
):
    del B_x
    q_t = A_q[0].T
    k_t = A_k[0].T
    v_t = A_v[0].T
    sk_t = A_shift_k.T
    wp = jnp.transpose(B_w_phi, (1, 2, 0))
    ft = jnp.asarray(_dft_table(), dtype=BF16)
    zero = jnp.asarray(np.zeros((128,), np.int32))

    hbm = pl.BlockSpec(memory_space=pl.ANY)
    spec = [pltpu.VMEM((C_ROWS[i + 1] - C_ROWS[i], NC * 384), F32) for i in range(4)]
    out_t = pl.pallas_call(
        _kernel,
        out_shape=jax.ShapeDtypeStruct((D, S), BF16),
        in_specs=[hbm] * 12,
        out_specs=hbm,
        scratch_shapes=[
            pltpu.VMEM((D, S), BF16),
            pltpu.VMEM((D, S), BF16),
            pltpu.VMEM((D, S), BF16),
            pltpu.VMEM((D, S), BF16),
            pltpu.VMEM((D, 3 * D), BF16),
            pltpu.VMEM((D, D), BF16),
            pltpu.VMEM((4, D), BF16),
            pltpu.VMEM((D,), BF16),
            pltpu.VMEM((D,), BF16),
            pltpu.VMEM((DH, DH, NH), BF16),
            pltpu.VMEM((256, 256), BF16),
            pltpu.SMEM((128,), jnp.int32),
            pltpu.VMEM((D, D), jnp.uint32),
            pltpu.VMEM((D // 2 + 8, D), jnp.uint32),
            pltpu.VMEM((D // 2, D), jnp.uint32),
            *spec, *spec,
            pltpu.VMEM((C_ROWS[3], NC * 256), F32),
            pltpu.VMEM((D - C_ROWS[3], NC * 256), F32),
            pltpu.VMEM((2 * NG, 48, 80), F32),
            pltpu.VMEM((2 * NG, 24, 80), jnp.uint32),
            pltpu.VMEM((D, S), F32),
            pltpu.VMEM((8, S), F32),
            pltpu.VMEM((D, S), BF16),
            pltpu.VMEM((5, D, 128), F32),
            pltpu.SemaphoreType.DMA((7,)),
        ],
        compiler_params=pltpu.CompilerParams(vmem_limit_bytes=100 * 1024 * 1024),
    )(q_t, k_t, v_t, A_ssm_k, B_wqkv, B_wo,
      sk_t, A_ssm_D, gate_w, wp, ft, zero)
    return out_t.T[None]
```

```python
import math

import jax
import jax.numpy as jnp
import numpy as np
import jax.experimental.pallas as pl
import jax.experimental.pallas.tpu as pltpu

S = 2048
D = 576
NH = 32
DH = 18
NG = 8
GR = 72
PR = 544
NC = 16
NIT = 4
CH = S // NIT
CB = 8
RO = 16
A_ROWS = (0, 160, 368, 576)
C_ROWS = (0, 32, 64, 512, 576)
RB = (C_ROWS[3] - C_ROWS[2]) // NIT
PW_QT, PW_Q, PW_N, PW_W, PW_WT = 1.12, (0, 0, 0, 0), (0, 0, 0.5, 0.68), (0.83, 0.94, 1.06, 1.02), 1.01
W3_ROWS = 544
GATE_AT = ((0, 1), (2,), (3,))
PB_VT, PB_V, PB_X, PB_KT, PB_K, PB_H = 2.5, (1.15, 0.81, 1.04, 0.91), 0, 1.01, (0,) * 4, 0
XS, XO, HO = 4, 0, 1
WPOS = (2, 3, 6, 7, 10)
WW = 12

F32 = jnp.float32
BF16 = jnp.bfloat16
_NN = (((1,), (0,)), ((), ()))
_NT = (((1,), (1,)), ((), ()))
LOG2E = math.log2(math.e)


def _dot(a, b, dn=_NN):
    return jax.lax.dot_general(a, b, dn, preferred_element_type=F32)


def _eps(c):
    return 1 if (c // 2) % 2 == 0 else -1


def _iota(shape, dim):
    return jax.lax.broadcasted_iota(jnp.int32, shape, dim)


def _cat(xs, axis=0):
    return jnp.concatenate(xs, axis=axis)


def _pk(x):
    return pltpu.bitcast(x, jnp.uint32)


def _upk(x):
    return pltpu.bitcast(x, BF16)


def _rcp(x):
    return pl.reciprocal(x, approx=True)


class _Wt:
    def __init__(self, ref, pos):
        self.ref, self.pos = ref, pos

    def put(self, r0, r1, val):
        for t, p in enumerate(self.pos):
            w = min(128, D - 128 * t)
            self.ref[r0:r1, 128 * p:128 * p + w] = val[:, 128 * t:128 * t + w]

    def main(self, r0, r1):
        return _upk(_cat([self.ref[r0:r1, 128 * p:128 * p + 128] for p in self.pos[0:4]], 1))

    def tail(self, r0, r1):
        return _upk(self.ref[r0:r1, 128 * self.pos[4]:128 * self.pos[4] + 64])


def _dft_table():
    om = np.pi * (2 * np.arange(128) + 1) / 256.0
    tau = np.arange(256)
    ang = np.outer(tau, om)
    return np.concatenate([np.cos(ang), -np.sin(ang)], axis=1).astype(np.float32)


class _Pacer:
    def __init__(self, mask):
        self.mask = mask
        self.runs = [[]]
        self.len = [0.0]

    def add(self, arr, cycles, w=1.0):
        if w == 0:
            if self.runs[-1]:
                self.runs.append([])
                self.len.append(0.0)
            return
        cycles = cycles * w
        n = arr.shape[0] // 8
        for r in range(n):
            self.runs[-1].append([self.len[-1] + cycles * r / n, arr, 8 * r, None])
        self.len[-1] += cycles

    def plan(self, sizes):
        tot, cap = float(sum(sizes)), sum(self.len)
        edges, acc = [], 0.0
        for ln in self.len:
            acc += ln
            edges.append(acc / cap * tot)
        self.unit_run, done = [], 0.0
        self.load = [0.0] * len(self.runs)
        for sz in sizes:
            r = min(i for i, e in enumerate(edges) if done + sz / 2 <= e + 1e-6)
            self.unit_run.append(r)
            self.load[r] += sz
            done += sz
        self.used = [0.0] * len(self.runs)
        self.unit = -1

    def next_unit(self):
        self.unit += 1

    def gate(self, x, nops):
        return jnp.where(self.mask, x, self.token(nops))

    def token(self, nops):
        r = self.unit_run[self.unit]
        t = self.len[r] * self.used[r] / self.load[r]
        self.used[r] += nops
        tok = [e for e in self.runs[r] if e[0] <= t][-1]
        if tok[3] is None:
            tok[3] = tok[1][tok[2]:tok[2] + 8, 0:128]
        return tok[3]


class _NoPacer:
    def add(self, arr, cycles, w=1.0):
        pass


def _expand(m, lo2):
    r = pltpu.roll(m, 2, 0)
    ab = jnp.where(lo2, m, r)
    cd = jnp.where(lo2, r, m)
    return [ab] * 4 + [cd] * 4 + [m]


def _feature_map(p, normalize):
    p = p.reshape(4, 17, 8, 128)
    sub = _iota((4, 8, 128), 1)
    sh = p[:, 0]
    v0 = []
    for gp in range(2):
        v8 = jnp.where(sub < 4, sh, 0.0) if gp == 0 else jnp.where(sub < 4, 0.0, sh)
        r8 = pltpu.roll(v8, 2, 1)
        v0 += [jnp.where(sub % 4 < 2, v8, r8), jnp.where(sub % 4 < 2, r8, v8)]
    vs = [jnp.stack(v0, axis=1).reshape(16, 8, 128)]
    pm = p[:, 1:17].reshape(16, 4, 8, 128)
    vs += [pm[:, j] for j in range(4)]

    def ext(op):
        r = op(op(op(op(vs[0], vs[1]), vs[2]), vs[3]), vs[4])
        r = op(r, pltpu.roll(r, 2, 1))
        return op(r, pltpu.roll(r, 4, 1))

    def tot(e):
        r = (e[1] + e[2]) + (e[3] + e[4])
        r = (r + e[0]) + pltpu.roll(r, 2, 1)
        return r + pltpu.roll(r, 4, 1)

    mx = ext(jnp.maximum)
    mn = ext(jnp.minimum)
    ep = [jnp.exp2(v - mx) for v in vs]
    em = [jnp.exp2(mn - v) for v in vs]
    if normalize:
        rp = _rcp(tot(ep))
        rm = _rcp(tot(em))
        ep = [e * rp for e in ep]
    else:
        rm = tot(ep) * _rcp(tot(em))
    em = [e * rm for e in em]
    out = _cat(ep[1:5] + em[1:5] + [ep[0], em[0]], 1)
    return [out[i].astype(BF16) for i in range(2 * NG)]


def _kernel(q_hbm, k_hbm, v_hbm, h_hbm, w_hbm, wo_hbm,
            sk_hbm, dd_hbm, gw_hbm, wp_hbm, ft_hbm, zero_hbm,
            out_hbm,
            q_v, k_v, v_v, h_v, w_v, wo_v, sk_ref, dd_ref, gw_ref, wp_ref, ft_ref, zero_s,
            wkv_t, wq_t, wo_t, st0, st1, st2, st3,
            x3a, x3b, xh3c, x3d, h3a, h3b, h3d, y2l, y2h, y2dl, y2dh, kvacc, kvt, b_t, g8, o_v, cb,
            sems):
    y2, y2d = (y2l, y2h), (y2dl, y2dh)
    wkv_t = _Wt(wkv_t, (0, 1, 2, 3, 4))
    wq_t = _Wt(wq_t, WPOS)
    wo_t = _Wt(wo_t, WPOS)

    x3s = ((x3a, 0), (x3b, 0), (xh3c, XO), (x3d, 0))
    h3s = ((h3a, 0), (h3b, 0), (xh3c, HO), (h3d, 0))

    def cp(src, dst, i):
        return pltpu.make_async_copy(src, dst, sems.at[i])

    def cq(i, s):
        return cp(q_hbm.at[:, CH * i:CH * (i + 1)], q_v.at[:, CH * i:CH * (i + 1)], s)

    def ca(i, s):
        rows = slice(A_ROWS[i], A_ROWS[i + 1])
        return [cp(h_hbm.at[rows, :], h_v.at[rows, :], s),
                cp(k_hbm.at[rows, :], k_v.at[rows, :], s),
                cp(v_hbm.at[rows, :], v_v.at[rows, :], s)]

    sets = [
        [cp(sk_hbm, sk_ref, 0), cp(dd_hbm, dd_ref, 0), cp(gw_hbm, gw_ref, 0), cp(wp_hbm, wp_ref, 0)],
        [cp(w_hbm.at[:, 512:1152], w_v.at[:, 512:1152], 1)],
        [cp(q_hbm.at[:, 0:256], q_v.at[:, 0:256], 2)],
        [cp(q_hbm.at[:, 256:CH], q_v.at[:, 256:CH], 3),
         cp(w_hbm.at[:, 1152:1728], w_v.at[:, 1152:1728], 3)],
        [cp(zero_hbm, zero_s, 4), cp(ft_hbm, ft_ref, 4), cq(1, 4)] + ca(0, 4),
        [cq(2, 5), cp(w_hbm.at[:, 0:512], w_v.at[:, 0:512], 5)] + ca(1, 5),
        [cq(3, 6), cp(wo_hbm, wo_v, 6)] + ca(2, 6),
    ]

    def c_out(i):
        return cp(o_v.at[RO * i:RO * (i + 1), :], out_hbm.at[RO * i:RO * (i + 1), :], 0)

    def wait(i):
        for c in sets[i]:
            c.wait()

    for cs in sets:
        for c in cs:
            c.start()
    wait(0)

    def row_maps(shape):
        r = _iota(shape, 0)
        j, s = r // 8, r % 8
        feat = jnp.where(j < 8, 4 * (j % 4) + s // 2, 16 + s // 4)
        head = jnp.where(j < 8, 2 * (j // 4) + s % 2, s % 4)
        return feat, head

    sk = sk_ref[...].astype(F32)
    for j in range(4):
        cb[j] = jnp.broadcast_to(sk[j:j + 1, :], (128, D)).T
    dd = dd_ref[...].astype(F32).reshape(1, D)
    cb[4] = jnp.broadcast_to(dd, (128, D)).T
    cb[5] = jnp.broadcast_to(gw_ref[...].astype(F32).reshape(1, D), (128, D)).T

    col = _iota((NH, 640), 1)
    hrow = _iota((NH, 640), 0) * DH
    wt = jnp.zeros((DH, 640), F32)
    for d in range(DH):
        sel = jnp.where(col == hrow + d, 1.0, 0.0).astype(BF16)
        wt = wt + _dot(wp_ref[d], sel)
    rsel = jnp.where(row_maps((GR, DH))[0] == _iota((GR, DH), 1), 1.0, 0.0).astype(BF16)
    z0 = _dot(rsel, wt.astype(BF16))
    z64 = pltpu.roll(z0, 64, 1)

    zrel = _iota((GR, 128), 1) - DH * row_maps((GR, 128))[1]

    def fold(z, off, base, dst):
        units = []
        for g in range(NG):
            units += [(g, 0, 32, off + GR * g, 36), (g, 32, 32, off + GR * g + 36, 36),
                      (g, 64, 8, off + GR * g, GR)]
        res = {}
        for t in range(5):
            us = [u for u in units if u[3] < 128 * (t + 1) and u[3] + u[4] > 128 * t]
            es = []
            for g, r0, nr, _, _ in us:
                rel = zrel[r0:r0 + nr] + (128 * t - off - GR * g)
                m = jnp.logical_and(rel >= 0, rel < DH)
                es.append(jnp.where(m, z[r0:r0 + nr, 128 * t:128 * t + 128], 0.0))
            if sum(u[2] for u in us) % 16:
                es.append(jnp.zeros((8, 128), F32))
            r = _dot(_cat(es).astype(BF16), w_v[:, base + 128 * t: base + 128 * (t + 1)], _NT)
            o = 0
            for u in us:
                res[u] = r[o:o + u[2]] + res[u] if u in res else r[o:o + u[2]]
                o += u[2]
        sw = _iota((8, D), 0)
        rows = []
        for p in range(NG // 2):
            shs = []
            for g in (2 * p, 2 * p + 1):
                ab, cd, v8 = (res[u] for u in units[3 * g: 3 * g + 3])
                m17 = jnp.where(sw < 4, pltpu.roll(v8, 4, 0), v8)
                ex = _expand(m17, sw % 4 < 2)
                rows += [ab - _cat(ex[0:4]), cd - _cat(ex[4:8])]
                shs.append(v8 - m17)
            rows.insert(5 * p, shs[0] + pltpu.roll(shs[1], 4, 0))
        for p in range(2):
            r = _cat(rows[10 * p: 10 * (p + 1)]) * LOG2E
            dst.put(PR // 4 * p, PR // 4 * (p + 1), _pk(r.astype(BF16)))

    wait(1)
    fold(z64, 64, 512, wkv_t)

    lane = _iota((16, 128), 1)
    sub8 = _iota((8, 128), 0)
    top = sub8 < 4

    def proj_steps(w_t, r0, r1, c0, pacer, wt_=1.0, wm=(1.0,) * 4, nt=4):
        m = 2 * (r1 - r0)
        rs = [r0 + (r1 - r0) * j * nt // 4 for j in range(4 // nt + 1)]
        tail = _cat([_dot(w_t.tail(a, b), q_v[512:D, pl.ds(c0, 128 * nt)])
                     for a, b in zip(rs[:-1], rs[1:])])
        pacer.add(tail, m, wt_)
        yield None
        for n in range(nt):
            cn = c0 + 128 * n
            if not isinstance(cn, int):
                cn = pl.multiple_of(cn, 128)
            pm_ = _dot(w_t.main(r0, r1), q_v[0:512, pl.ds(cn, 128)])
            pacer.add(pm_, m, wm[n])
            yield pm_ + tail[:, 128 * n:128 * n + 128]

    def k_feat(pk):
        return _feature_map(pk, True)

    ones8 = jnp.ones((8, 128), F32)

    def v_ext(pv):
        out = []
        for g in range(NG):
            out.append(_cat([pv[GR * g: GR * g + 40], ones8]).astype(BF16))
            out.append(_cat([pv[GR * g + 32: GR * g + 72], ones8]).astype(BF16))
        return out

    def kv_step(acc, phi, vx):
        r = [_dot(vx[p], phi[p], _NT) for p in range(2 * NG)]
        return r if acc is None else [a + b for a, b in zip(acc, r)]

    def spec_put(refs, row, tiles):
        i = [j for j in range(4) if row < C_ROWS[j + 1]][0]
        r8 = (row - C_ROWS[i]) // 8
        ref, slot = refs[i]
        ref[pl.ds(zero_s[0] + r8 if i < 2 else r8, 2), :, :, slot] = jnp.stack(
            [t.reshape(2, 8, 128) for t in tiles], axis=1).reshape(2, NC, 3, 8, 128)

    def h_spec(rows16, pacer, gpacer):
        le, lo_ = [], []
        for r in rows16:
            hr = h_v[r:r + 16, :]
            for c in range(NC):
                (le if c % 2 == 0 else lo_).append(hr[:, 128 * c:128 * c + 128])
        he = _dot(_cat(le), ft_ref[0:128, :])
        ho = _dot(_cat(lo_), ft_ref[128:256, :])
        gpacer.add(ho, 128 * len(rows16))
        gpacer.add(ho, 0, 0)
        pacer.add(he, 64 * len(rows16), PB_H)
        pacer.add(ho, 64 * len(rows16), PB_H)
        for sb, r in enumerate(rows16):
            tiles = []
            prev = None
            for c in range(NC):
                o = (sb * (NC // 2) + c // 2) * 16
                hh = (he if c % 2 == 0 else ho)[o:o + 16]
                if prev is None:
                    cc = hh[:, 0:128] + cb[4, r:r + 16, :]
                    dd_ = hh[:, 128:256]
                else:
                    hp = hh + prev if _eps(c) * _eps(c - 1) > 0 else hh - prev
                    cc = hp[:, 0:128]
                    dd_ = hp[:, 128:256]
                prev = hh
                tiles += [cc, cc + dd_, dd_ - cc]
            spec_put(h3s, r, tiles)

    def x_spec(rows16, pacer):
        le, lo_ = [], []
        for r in rows16:
            s0, s1, s2, s3 = (cb[j, r:r + 16, :] for j in range(4))
            pr1 = None
            pr2 = None
            kr_ = k_v[r:r + 16, :].astype(F32)
            vr_ = v_v[r:r + 16, :].astype(F32)
            for c in range(NC):
                cs = slice(128 * c, 128 * c + 128)
                kf = kr_[:, cs]
                r1 = pltpu.roll(kf, 1, 1)
                k1 = jnp.where(lane >= 1, r1, 0.0 if pr1 is None else pr1)
                pr1 = r1
                w1 = s0 * kf + s1 * k1
                w2 = s2 * kf + s3 * k1
                r2 = pltpu.roll(w2, 2, 1)
                k2 = jnp.where(lane >= 2, r2, 0.0 if pr2 is None else pr2)
                pr2 = r2
                kv = ((w1 + k2) * vr_[:, cs]).astype(BF16)
                (le if c % 2 == 0 else lo_).append(kv)
        xe = _dot(_cat(le), ft_ref[0:128, :])
        xo = _dot(_cat(lo_), ft_ref[128:256, :])
        pacer.add(xe, 64 * len(rows16), PB_X)
        pacer.add(xo, 64 * len(rows16), PB_X)
        for sb, r in enumerate(rows16):
            tiles = []
            for c in range(NC):
                o = (sb * (NC // 2) + c // 2) * 16
                xx = (xe if c % 2 == 0 else xo)[o:o + 16]
                xa = xx[:, 0:128]
                xb = xx[:, 128:256]
                tiles += [xa + xb, xb, xa]
            spec_put(x3s, r, tiles)

    def conv(x3, h3, r_in, r_out, ntask, pacer, y2=y2):
        steps = [(t0, comp, s) for t0 in range(0, NC, CB) for comp in range(3) for s in range(t0 + CB)]
        pacer.plan([3 * CB * (2 * t0 + CB + 1) for t0 in range(0, NC, CB)] * ntask)
        toks = []
        for tk in range(ntask):
            toks.append([])
            for t0, comp, s in steps:
                if comp == 0 and s == 0:
                    pacer.next_unit()
                toks[-1].append(pacer.token(2 * (t0 + CB - max(s, t0))))
        rows = pl.ds(r_in, ntask)
        outs = []
        for i, (t0, comp, s) in enumerate(steps):
            if s == 0:
                xs_, hh = (ref[rows, 0:t0 + CB, comp, slot] for ref, slot in (x3, h3))
                hh = [hh[:, j] for j in range(t0 + CB)]
                if comp == 1:
                    k1 = acc
                acc = {} if comp == 0 else dict(k1)
            x = jnp.where(pacer.mask, xs_[:, s], jnp.stack([tk[i] for tk in toks]))
            for t in range(max(s, t0), t0 + CB):
                sg = _eps(s) * _eps(t - s) * _eps(t) * (-1 if comp == 1 else 1)
                prod = x * hh[t - s]
                if t not in acc:
                    acc[t] = prod
                elif sg > 0:
                    acc[t] = acc[t] + prod
                else:
                    acc[t] = acc[t] - prod
            if comp > 0 and s >= t0:
                outs.append(acc[s])
            if len(outs) == 2 * CB:
                y2[t0 // CB][pl.ds(r_out, ntask)] = jnp.stack(outs, axis=1)
                outs = []

    def gate(c, pacer):
        for n in range(CH // 128):
            pacer.next_unit()
            cs = slice(CH * c + 128 * n, CH * c + 128 * (n + 1))
            acc = None
            qf = q_v[:, cs].astype(F32)
            gb = cb[5]
            for j in range(D // 16):
                w = _cat([pacer.gate(gb[16 * j + r:16 * j + r + 8, :], 1) for r in (0, 8)])
                t = qf[16 * j:16 * j + 16] * w
                acc = t if acc is None else acc + t
            s = acc[0:8] + acc[8:16]
            for sh in (4, 2, 1):
                s = s + pltpu.roll(s, sh, 0)
            g = 1.0 / (1.0 + jnp.exp(-s))
            g8[0:8, cs] = g * (1.0 / 128.0)
            g8[8:16, cs] = 1.0 - g

    def true_mask():
        return jnp.abs(ft_ref[0:16, 0:128].astype(F32)[0:8]) < 2.0

    nop = _NoPacer()

    wait(2)
    pks = list(proj_steps(wkv_t, 0, PR // 2, 0, nop, nt=2))[1:]
    phis = [k_feat(pks[0])]
    wait(3)
    phis.append(k_feat(pks[1]))
    phis += [k_feat(pk) for pk in list(proj_steps(wkv_t, 0, PR // 2, 256, nop, nt=2))[1:]]
    wkv_t.put(PR // 2, (PR + D) // 2, _pk(w_v[:, 2 * D:3 * D].T))
    vxs = [v_ext(pv) for pv in list(proj_steps(wkv_t, PR // 2, (PR + D) // 2, 0, nop))[1:]]
    for p in range(2 * NG):
        kvacc[p] = _dot(_cat([v[p] for v in vxs], 1), _cat([f[p] for f in phis], 1), _NT)

    for b in range(3):
        wait(4 + b)
        ntask = (C_ROWS[b] - C_ROWS[b - 1]) // 8 if b > 0 else 0
        pacer = _Pacer(true_mask())
        gpacer = _Pacer(true_mask())
        r16 = list(range(A_ROWS[b], A_ROWS[b + 1], 16))
        parts = [r16[(len(r16) * n) // 4: (len(r16) * (n + 1)) // 4] for n in range(4)]
        vs = proj_steps(wkv_t, PR // 2, (PR + D) // 2, CH * (b + 1), pacer, PB_VT, PB_V)
        ks = proj_steps(wkv_t, 0, PR // 2, CH * (b + 1), pacer, PB_KT, PB_K)
        next(vs)
        vxs = [v_ext(next(vs))]
        for n in range(3):
            vxs.append(v_ext(next(vs)))
            x_spec(parts[n], pacer)
        next(ks)
        x_spec(parts[3], pacer)
        acc = None
        phi = None
        for n in range(4):
            nxt = k_feat(next(ks))
            if n > 0:
                acc = kv_step(acc, phi, vxs[n - 1])
            phi = nxt
            h_spec(parts[n], pacer, gpacer)
        acc = kv_step(acc, phi, vxs[3])
        for p in range(2 * NG):
            kvacc[p] += acc[p]
        if not ntask:
            gpacer = pacer
        gpacer.plan([D // 8] * (4 * len(GATE_AT[b])))
        for c in GATE_AT[b]:
            gate(c, gpacer)
        if b == 2:
            fold(z0, 0, 0, wq_t)
            wo_t.put(0, D // 2, _pk(wo_v[...].T))
        if ntask:
            conv(x3s[b - 1], h3s[b - 1], 0, zero_s[0] + C_ROWS[b - 1] // 8, ntask, pacer)

    kr = _iota((48, 80), 0)
    kc = _iota((48, 80), 1)
    plus = jnp.logical_or(kc < 32, jnp.logical_and(kc >= 64, kc < 72))
    epsm = jnp.where(jnp.logical_and(kr >= 40, plus), 1e-6, 0.0)
    for pp in range(2):
        rv = kr - 4 * pp
        rhead = jnp.where(kr >= 40, (kr - 40) // 4, jnp.where(rv >= DH, 1, 0))
        rok = jnp.logical_or(kr >= 40, jnp.logical_and(rv >= 0, rv < 2 * DH))
        cok = jnp.logical_or(kc < 64, (kc % 4) // 2 == pp)
        keep = jnp.logical_and(jnp.logical_and(rok, cok), rhead == kc % 2)
        for g in range(NG):
            p = 2 * g + pp
            kvt[p] = _pk(jnp.where(keep, kvacc[p] + epsm, 0.0).astype(BF16))

    def loop2(i2, carry):
        pacer = _Pacer(true_mask())
        for hf in range(2):
            q_side(2 * i2 + hf, pacer, hf == 1)
        conv(x3s[2], h3s[2], i2 * (2 * RB // 8), i2 * (2 * RB // 8) + C_ROWS[2] // 8, 2 * RB // 8, pacer)
        return carry

    def q_side(i, pacer, last):
        c0 = pl.multiple_of(i * CH, CH)

        def sub(n):
            return pl.ds(pl.multiple_of(c0 + 128 * n, 128), 128)

        def numden(n, pq):
            omg = g8[8:16, sub(n)]
            ov = []
            tiles = _feature_map(pq, False)
            for gi in range(NG):
                res = []
                for pp in range(2):
                    a = _dot(_upk(kvt[2 * gi + pp]), tiles[2 * gi + pp])
                    if pp == 1 and gi % 2 == 1:
                        pacer.add(a, 48, PW_N[n])
                    r = omg * _rcp(a[40:48])
                    r4 = pltpu.roll(r, 4, 0)
                    ra = jnp.where(top, r, r4)
                    rb = jnp.where(top, r4, r)
                    mix = jnp.where(sub8 < 2 + 4 * pp, ra, rb)
                    res.append([a[8 * j:8 * j + 8] * s for j, s in enumerate((ra, ra, mix, rb, rb))])
                ov += res[0][0:4] + [res[0][4] + res[1][0]] + res[1][1:5]
            return _cat(ov[0:64]).astype(BF16), _cat(ov[64:72]).astype(BF16)

        def park(n, val):
            st = (st0, st1, st2, st3)[n]
            cs = slice(128 * (2 + n % 2), 128 * (3 + n % 2))
            st[pl.ds(pl.multiple_of(zero_s[0], 8), D), cs] = val
            return st[:, cs]

        def womain(n, o):
            bb = _dot(wo_t.main(0, D // 2), o[0])
            nr = W3_ROWS if (n == 3 and last) else D
            pacer.add(bb[0:nr], nr, PW_W[n])
            return park(n, bb) if n < 3 else bb

        qs = proj_steps(wq_t, 0, PR // 2, c0, pacer, PW_QT, PW_Q)
        next(qs)
        pq0 = next(qs)
        pq1 = next(qs)
        o0 = numden(0, pq0)
        pq2 = next(qs)
        o1 = numden(1, pq1)
        b0 = womain(0, o0)
        pq3 = next(qs)
        o2 = numden(2, pq2)
        b1 = womain(1, o1)
        o3 = numden(3, pq3)
        b2 = womain(2, o2)
        btail = _dot(wo_t.tail(0, D // 2), _cat([o[1] for o in (o0, o1, o2, o3)], 1))
        pacer.add(btail, 576, PW_WT)
        b_t[:, pl.ds(c0, 384)] = _cat([b0, b1, b2], 1) + btail[:, 0:384]
        bt3 = park(3, btail[:, 384:512])
        b_t[:, sub(3)] = womain(3, o3) + bt3

    jax.lax.fori_loop(0, NIT // 2, loop2, 0)

    pacer = _Pacer(true_mask())
    for i in range(D // RO):
        rows = slice(RO * i, RO * (i + 1))
        if RO * i == C_ROWS[3]:
            z = zero_s[0]
            conv(x3s[3], h3s[3], 0, z, (C_ROWS[4] - C_ROWS[3]) // 8, pacer, y2d)
        ysrc, y0 = (y2, RO * i) if RO * i < C_ROWS[3] else (y2d, RO * i - C_ROWS[3])
        yy = [y[y0 // 8: (y0 + RO) // 8] for y in ysrc]
        ye, yo = (_cat([_cat([yy[c // CB][:, CB * comp + c % CB].reshape(RO, 128) for comp in range(2)], 1)
                        for c in range(par, NC, 2)]) for par in range(2))
        te = _dot(ye.astype(BF16), ft_ref[0:128, :], _NT)
        to = _dot(yo.astype(BF16), ft_ref[128:256, :], _NT)
        if RO * (i + 2) <= C_ROWS[3]:
            pacer.add(to, 8 * RO)
        y = _cat([(te if c % 2 == 0 else to)[(c // 2) * RO: (c // 2 + 1) * RO] for c in range(NC)], 1)
        gq = q_v[rows, :].astype(F32) * _cat([g8[0:8, :]] * (RO // 8))
        o_v[rows, :] = (gq * y + b_t[rows, :]).astype(BF16)
        c_out(i).start()
    for i in range(D // RO):
        c_out(i).wait()


@jax.jit
def pallas_gated_mix__ssm_conv_h3__linear_kernel_hedgehog__prompt_kernel(
    A_q: jax.Array,
    A_k: jax.Array,
    A_v: jax.Array,
    A_shift_k: jax.Array,
    A_ssm_k: jax.Array,
    A_ssm_D: jax.Array,
    B_x: jax.Array,
    B_wqkv: jax.Array,
    B_w_phi: jax.Array,
    B_wo: jax.Array,
    gate_w: jax.Array,
):
    del B_x
    q_t = A_q[0].T
    k_t = A_k[0].T
    v_t = A_v[0].T
    sk_t = A_shift_k.T
    wp = jnp.transpose(B_w_phi, (1, 2, 0))
    ft = jnp.asarray(_dft_table(), dtype=BF16)
    zero = jnp.asarray(np.zeros((128,), np.int32))

    hbm = pl.BlockSpec(memory_space=pl.ANY)
    spec = [pltpu.VMEM(((C_ROWS[i + 1] - C_ROWS[i]) // 8, NC, 3, XS if i == 2 else 1, 8, 128), F32)
            for i in range(4)]
    out_t = pl.pallas_call(
        _kernel,
        out_shape=jax.ShapeDtypeStruct((D, S), BF16),
        in_specs=[hbm] * 12,
        out_specs=hbm,
        scratch_shapes=[
            pltpu.VMEM((D, S), BF16),
            pltpu.VMEM((D, S), BF16),
            pltpu.VMEM((D, S), BF16),
            pltpu.VMEM((D, S), BF16),
            pltpu.VMEM((D, 3 * D), BF16),
            pltpu.VMEM((D, D), BF16),
            pltpu.VMEM((4, D), BF16),
            pltpu.VMEM((D,), BF16),
            pltpu.VMEM((D,), BF16),
            pltpu.VMEM((DH, DH, NH), BF16),
            pltpu.VMEM((256, 256), BF16),
            pltpu.SMEM((128,), jnp.int32),
            pltpu.VMEM(((PR + D) // 2, D), jnp.uint32),
            pltpu.VMEM((PR // 2, 128 * WW), jnp.uint32),
            pltpu.VMEM((D // 2, 128 * WW), jnp.uint32),
            *[pltpu.VMEM((D, 512), F32)] * 4,
            *spec,
            spec[0], spec[1], spec[3],
            *[pltpu.VMEM((C_ROWS[3] // 8, 2 * CB, 8, 128), F32)] * 2,
            *[pltpu.VMEM(((D - C_ROWS[3]) // 8, 2 * CB, 8, 128), F32)] * 2,
            pltpu.VMEM((2 * NG, 48, 80), F32),
            pltpu.VMEM((2 * NG, 24, 80), jnp.uint32),
            pltpu.VMEM((D, S), F32),
            pltpu.VMEM((16, S), F32),
            pltpu.VMEM((D, S), BF16),
            pltpu.VMEM((6, D, 128), F32),
            pltpu.SemaphoreType.DMA((7,)),
        ],
        compiler_params=pltpu.CompilerParams(vmem_limit_bytes=100 * 1024 * 1024),
    )(q_t, k_t, v_t, A_ssm_k, B_wqkv, B_wo,
      sk_t, A_ssm_D, gate_w, wp, ft, zero)
    return out_t.T[None]
```
